```python
import jax
import jax.numpy as jnp

def _softmax(x, axis=-1):
    return jax.nn.softmax(x, axis=axis)

def _gelu(x):
    return jax.nn.gelu(x, approximate=True)

def _silu(x):
    return jax.nn.silu(x)

def _sigmoid(x):
    return jax.nn.sigmoid(x)

def _layernorm(x, axis=-1, eps=1e-05):
    m = jnp.mean(x, axis=axis, keepdims=True)
    v = jnp.var(x, axis=axis, keepdims=True)
    return (x - m) / jnp.sqrt(v + eps)

def _scatter_add(tgt, idx, src, axis=0):
    return tgt.at[idx].add(src)

def _segment_sum(src, seg, n):
    return jax.ops.segment_sum(src, seg, n)

class _Rng:

    def __init__(self, key):
        self._k = key

    def _next(self):
        self._k, sub = jax.random.split(self._k)
        return sub

    def normal(self, shape):
        return jax.random.normal(self._next(), shape, dtype=jnp.bfloat16)

    def randint(self, lo, hi, shape):
        return jax.random.randint(self._next(), shape, lo, hi, dtype=jnp.int32)

    def uniform(self, shape, lo=0.0, hi=1.0):
        return jax.random.uniform(self._next(), shape, jnp.bfloat16, lo, hi)

    def permutation(self, n):
        return jax.random.permutation(self._next(), n)
kernel_name = 'adaLN_cond__sliding_block_cached__dense_activation_gelu__decode'

def setup_inputs():
    _rng = _Rng(jax.random.key(int.from_bytes(__import__("os").urandom(4), "little")))
    _w = lambda a: (lambda t: t.astype(jnp.bfloat16) if jnp.issubdtype(t.dtype, jnp.floating) else t)(jnp.asarray(a))

    def _A_setup():
        B, Sq, D = (4, 1, 640)
        Hq, Hkv, Sk, Dh = (32, 32, 8192, 128)
        assert Hq % Hkv == 0, (Hq, Hkv)
        return {'x': _w((lambda *s: _rng.normal(s) * 0.05)(B, Sq, D)), 'k_cache': _w((lambda *s: _rng.normal(s) * 0.05)(B, Hkv, Sk, Dh)), 'v_cache': _w((lambda *s: _rng.normal(s) * 0.05)(B, Hkv, Sk, Dh)), 'wq': _w((lambda *s: _rng.normal(s) * 0.05)(D, Hq * Dh) * D ** (-0.5)), 'wo': _w((lambda *s: _rng.normal(s) * 0.05)(Hq * Dh, D) * (Hq * Dh) ** (-0.5))}
    _A_in = _A_setup()

    def _B_setup():
        B, S, D, F = (4, 1, 640, 1728)
        return {'x': _w((lambda *s: _rng.normal(s) * 0.05)(B, S, D)), 'w1': _w((lambda *s: _rng.normal(s) * 0.05)(D, F) * D ** (-0.5)), 'b1': _w((lambda *s: _rng.normal(s) * 0.05)(F) * 0.01), 'w2': _w((lambda *s: _rng.normal(s) * 0.05)(F, D) * F ** (-0.5)), 'b2': _w((lambda *s: _rng.normal(s) * 0.05)(D) * 0.01)}
    _B_in = _B_setup()
    return {'A_x': _A_in['x'], 'A_k_cache': _A_in['k_cache'], 'A_v_cache': _A_in['v_cache'], 'A_wq': _A_in['wq'], 'A_wo': _A_in['wo'], 'B_x': _B_in['x'], 'B_w1': _B_in['w1'], 'B_b1': _B_in['b1'], 'B_w2': _B_in['w2'], 'B_b2': _B_in['b2'], 'c': _w((lambda *s: _rng.normal(s) * 0.05)(4, 640)), 'w_mod': _w((lambda *s: _rng.normal(s) * 0.05)(640, 6 * 640) * 640 ** (-0.5))}

def reference(A_x, A_k_cache, A_v_cache, A_wq, A_wo, B_x, B_w1, B_b1, B_w2, B_b2, c, w_mod):

    def _A_ref(x, k_cache, v_cache, wq, wo):
        B, Sq, D = x.shape
        Hq, Dh = (32, 128)
        Hkv, Sk = (k_cache.shape[1], k_cache.shape[2])
        W = min(4096, max(256, Sk // 4))
        rep = Hq // Hkv
        q = (lambda x, *d: x.transpose(*d))((x @ wq).reshape(B, Sq, Hq, Dh), 0, 2, 1, 3)
        k = jnp.repeat(k_cache[:, :, Sk - W:, :], rep, axis=1)
        v = jnp.repeat(v_cache[:, :, Sk - W:, :], rep, axis=1)
        scores = jnp.einsum('bhqd,bhkd->bhqk', q, k) * Dh ** (-0.5)
        p = _softmax(scores, axis=-1)
        o = jnp.einsum('bhqk,bhkd->bhqd', p, v)
        return (lambda x, *d: x.transpose(*d))(o, 0, 2, 1, 3).reshape(B, Sq, Hq * Dh) @ wo

    def _B_ref(x, w1, b1, w2, b2):
        h = jnp.einsum('bsd,df->bsf', x, w1) + b1
        h = _gelu(h)
        return jnp.einsum('bsf,fd->bsd', h, w2) + b2
    x = A_x
    mod = (_silu(c) @ w_mod).reshape(c.shape[0], 6, 1, -1)
    sa, ca, ga, sb, cb, gb = (mod[:, 0].copy(), mod[:, 1].copy(), mod[:, 2].copy(), mod[:, 3].copy(), mod[:, 4].copy(), mod[:, 5].copy())
    h = _layernorm(x, axis=-1) * (1 + ca) + sa
    x = x + ga * _A_ref(h, A_k_cache, A_v_cache, A_wq, A_wo)
    h = _layernorm(x, axis=-1) * (1 + cb) + sb
    x = x + gb * _B_ref(h, B_w1, B_b1, B_w2, B_b2)
    return x
```

```python
import functools

import jax
import jax.numpy as jnp
from jax import lax
import jax.experimental.pallas as pl
import jax.experimental.pallas.tpu as pltpu

F32 = jnp.float32
BF16 = jnp.bfloat16

T = 128
LOOK = 8
RING = 16
EPS = 1e-5


def _nn(a, b):
    return lax.dot_general(a, b, (((1,), (0,)), ((), ())), preferred_element_type=F32)


def _nt(a, b):
    return lax.dot_general(a, b, (((1,), (1,)), ((), ())), preferred_element_type=F32)


def _layernorm(x):
    m = jnp.mean(x, axis=-1, keepdims=True)
    d = x - m
    v = jnp.mean(d * d, axis=-1, keepdims=True)
    return d * lax.rsqrt(v + EPS)


def _dup(x):
    return jnp.concatenate([x, x], axis=0)


def _kernel(x_hbm, c_hbm, b1_hbm, b2_hbm, k_hbm, v_hbm, wq_hbm, wo_hbm, w1t_hbm, w2_hbm, wm_hbm,
            out_ref,
            xb, cb, b1b, b2b, kv, wq, wo, w1t, w2, wm, s_ref, h_ref, y_ref, mod_ref,
            kv_sem, wq_sem, wo_sem, misc_sem, w2_sem, *, win):
    nb, nh, sk, dh = k_hbm.shape
    d = x_hbm.shape[1]
    f = w2_hbm.shape[0]
    ng = nh // 2
    nj = win // T
    row0 = sk - win
    nd = d // T
    scale = dh ** -0.5
    SM_X, SM_C, SM_B1, SM_B2, SM_MA, SM_MB, SM_W1 = range(7)

    def kv_copy(which, g, j, t):
        hh, r = t // 4, (t % 4) * 32
        src = (k_hbm, v_hbm)[which]
        return pltpu.make_async_copy(
            src.at[:, 2 * g + hh, pl.ds(row0 + j * T + r, 32), :],
            kv.at[j, which, hh, :, pl.ds(r, 32), :], kv_sem.at[j])

    def tile_copy(src, dst, sem, r, c, nr=T):
        return pltpu.make_async_copy(src.at[pl.ds(r, nr), pl.ds(c, T)],
                                     dst.at[pl.ds(r, nr), pl.ds(c, T)], sem)

    def wq_copy(g, t):
        col = pl.multiple_of((2 * g + t // nd) * T, T)
        return tile_copy(wq_hbm, wq, wq_sem.at[g], (t % nd) * T, col)

    def wo_copy(g, t):
        row = pl.multiple_of((2 * g + t // nd) * T, T)
        return tile_copy(wo_hbm, wo, wo_sem.at[g], row, (t % nd) * T)

    def wait_all(ref, sem):
        pltpu.make_async_copy(ref, ref, sem).wait()

    nf = pl.cdiv(f, T)
    f_rows = [(i * T, min(T, f - i * T)) for i in range(nf)]

    ffn_copies = ([functools.partial(tile_copy, w1t_hbm, w1t, misc_sem.at[SM_W1], r, c * T, n)
                   for r, n in f_rows for c in range(nd)]
                  + [functools.partial(tile_copy, w2_hbm, w2, w2_sem.at[i], r, c * T, n)
                     for i, (r, n) in enumerate(f_rows) for c in range(nd)])

    def modb_start(j, t):
        n = j * 8 + t

        @pl.when(n < 4 * nd * nd)
        def _():
            row = pl.multiple_of((n % nd) * T, T)
            col = pl.multiple_of((2 * nd + n // nd) * T, T)
            tile_copy(wm_hbm, wm, misc_sem.at[SM_MB], row, col).start(priority=1)

    rows = lax.broadcasted_iota(jnp.int32, (8, T), 0)

    def step(j, carry, q, m, issue):
        mx, l, acc = carry
        if q is not None and m is not None:
            wait_all(kv.at[j], kv_sem.at[j])
        else:
            wait_all(kv.at[j, 0 if m is None else 1], kv_sem.at[j])
        if m is not None:
            p = jnp.exp(s_ref[j] - m)
            l = l + p
            p = p.astype(BF16)
        s = o = None
        for t in range(8):
            issue(t)
            if q is not None:
                r = _nt(q, kv[j, 0, t // 4, t % 4])
                s = r if s is None else jnp.where(rows == t, r, s)
            if m is not None:
                r = _nn(p, kv[j, 1, t // 4, t % 4])
                o = r if o is None else jnp.where(rows == t, r, o)
        if q is not None:
            s = s * scale
            s_ref[j] = s
            mx = jnp.maximum(mx, s)
        if m is not None:
            acc = acc + o
        return mx, l, acc

    def issue_first(j):
        def issue(t):
            kv_copy(0, 0, j, t).start(priority=0)
            modb_start(j, t)
        return issue

    def issue_mid(g, j):
        def issue(t):
            kv_copy(0, g, j, t).start(priority=0)
            kv_copy(1, g - 1, j, t).start(priority=1)
        return issue

    def init():
        return (jnp.full((8, T), -jnp.inf, F32), jnp.zeros((8, T), F32), jnp.zeros((8, T), F32))

    def project_q(g, starts):
        wq_g = wq.at[:, pl.ds(pl.multiple_of(2 * g * T, 2 * T), 2 * T)]
        wait_all(wq_g, wq_sem.at[g])
        h = h_ref[...].astype(BF16)
        res = []
        for hh in range(2):
            r = None
            for kk in range(nd):
                starts.pop(0)()
                z = _nn(h[:, kk * T:(kk + 1) * T], wq_g[kk * T:(kk + 1) * T, hh * T:(hh + 1) * T])
                r = z if r is None else r + z
            res.append(r)
        return jnp.where(rows < 4, res[0], res[1]).astype(BF16)

    def project_o(g, l, acc, starts):
        wo_g = wo.at[pl.ds(pl.multiple_of(2 * g * T, 2 * T), 2 * T), :]
        wait_all(wo_g, wo_sem.at[g])
        o = (acc / jnp.sum(l, axis=-1, keepdims=True)).astype(BF16)
        for cc in range(nd):
            res = []
            for hh in range(2):
                starts.pop(0)()
                res.append(_nn(o, wo_g[hh * T:(hh + 1) * T, cc * T:(cc + 1) * T]))
            y_ref[:, cc * T:(cc + 1) * T] += jnp.where(rows < 4, res[0], res[1])

    def starts_of(fn, g, prio0=0):
        return [functools.partial(lambda t: fn(g, t).start(priority=(t + prio0) % 2), t)
                for t in range(2 * nd)]

    def nops():
        return [lambda: None] * (2 * nd)

    def rowmax(mx):
        return jnp.max(mx, axis=-1, keepdims=True)

    def mod_a_start(n, _):
        col = pl.multiple_of(n * T, T)
        for r in range(nd):
            tile_copy(wm_hbm, wm, misc_sem.at[SM_MA], r * T, col).start(priority=r % 2)
            tile_copy(wm_hbm, wm, misc_sem.at[SM_MA], r * T, col + d).start(priority=(r + 1) % 2)
        return _

    lax.fori_loop(0, 1, mod_a_start, 0)
    small = [pltpu.make_async_copy(s, t, misc_sem.at[i]) for s, t, i in
             ((x_hbm, xb, SM_X), (c_hbm, cb, SM_C), (b1_hbm, b1b, SM_B1), (b2_hbm, b2b, SM_B2))]
    for cp in small:
        cp.start()
    lax.fori_loop(1, nd, mod_a_start, 0)
    for st in starts_of(wq_copy, 0):
        st()

    def first_issue(j, _):
        for t in range(8):
            issue_first(j)(t)
        return _

    lax.fori_loop(0, LOOK, first_issue, 0)

    for cp in small:
        cp.wait()
    wait_all(wm.at[:, pl.ds(0, 2 * d)], misc_sem.at[SM_MA])
    x = _dup(xb[...].astype(F32))
    cf = _dup(cb[...].astype(F32))
    sc = (cf * jax.nn.sigmoid(cf)).astype(BF16)
    mod_a = _nn(sc, wm[:, 0:2 * d])
    h_ref[...] = _layernorm(x) * (1.0 + mod_a[:, d:]) + mod_a[:, :d]
    y_ref[...] = jnp.zeros_like(y_ref)

    q = project_q(0, starts_of(wq_copy, 1))
    for st in starts_of(wo_copy, 0):
        st()
    carry = lax.fori_loop(
        0, nj - LOOK, lambda j, cr: step(j, cr, q, None, issue_first(j + LOOK)), init())
    carry = lax.fori_loop(
        nj - LOOK, nj, lambda j, cr: step(j, cr, q, None, issue_mid(1, j + LOOK - nj)), carry)

    wait_all(wm.at[:, pl.ds(2 * d, 4 * d)], misc_sem.at[SM_MB])
    mod_ref[...] = _nn(sc, wm[:, 2 * d:])

    def mid_issue(g, j):
        i = g * nj + j + LOOK
        return issue_mid(i // nj, i % nj)

    def phase(g, carry):
        mx, l, acc = carry
        q = project_q(g, starts_of(wq_copy, g + 1))

        @pl.when(g >= 2)
        def _():
            project_o(g - 2, l, acc, starts_of(wo_copy, g))

        @pl.when(g < 2)
        def _():
            for st in starts_of(wo_copy, g):
                st()

        m = rowmax(mx)
        return lax.fori_loop(0, nj, lambda j, cr: step(j, cr, q, m, mid_issue(g, j)), init())

    mx, l, acc = lax.fori_loop(1, ng - 1, phase, carry)

    g = ng - 1
    ffn = list(ffn_copies)

    def ffn_starts(n):
        return [functools.partial(lambda cp, p: cp().start(priority=p), ffn.pop(0), i % 2)
                for i in range(n)]

    def issue_last(j):
        def issue(t):
            kv_copy(1, ng - 1, j, t).start(priority=t % 2)
        return issue

    q = project_q(g, starts_of(wo_copy, g))
    project_o(g - 2, l, acc, ffn_starts(2 * nd))
    m = rowmax(mx)
    carry = lax.fori_loop(
        0, nj - LOOK, lambda j, cr: step(j, cr, q, m, issue_mid(g, j + LOOK)), init())

    def issue_last2(j):
        def issue(t):
            kv_copy(1, ng - 1, j, t).start(priority=0)
        return issue

    mx, l, acc = lax.fori_loop(
        nj - LOOK, nj, lambda j, cr: step(j, cr, q, m, issue_last(j + LOOK - nj)), carry)

    project_o(ng - 2, l, acc, ffn_starts(2 * nd))
    m = rowmax(mx)
    carry = lax.fori_loop(
        0, nj - LOOK, lambda j, cr: step(j, cr, None, m, issue_last(j + LOOK)), init())
    for st in ffn_starts(len(ffn)):
        st()
    mx, l, acc = lax.fori_loop(
        nj - LOOK, nj, lambda j, cr: step(j, cr, None, m, lambda t: None), carry)
    project_o(ng - 1, l, acc, nops())

    y = y_ref[...]
    y = y + pltpu.roll(y, 4, 0)
    ga, sb, cbm, gb = (mod_ref[:, i * d:(i + 1) * d] for i in range(4))
    x1 = x + ga * y
    h2 = (_layernorm(x1) * (1.0 + cbm) + sb).astype(BF16)
    wait_all(w1t, misc_sem.at[SM_W1])
    a = _nt(h2, w1t[...]) + b1b[...].astype(F32).reshape(1, f)
    a = jax.nn.gelu(a, approximate=True).astype(BF16)
    z = jnp.broadcast_to(b2b[...].astype(F32).reshape(1, d), (8, d))
    for i, (r, n) in enumerate(f_rows):
        wait_all(w2.at[pl.ds(r, n), :], w2_sem.at[i])
        z = z + _nn(a[:, r:r + n], w2[r:r + n, :])
    out_ref[...] = (x1 + gb * z)[0:4].astype(out_ref.dtype)


@jax.jit
def pallas_adaLN_cond__sliding_block_cached__dense_activation_gelu__decode_kernel(
    A_x: jax.Array,
    A_k_cache: jax.Array,
    A_v_cache: jax.Array,
    A_wq: jax.Array,
    A_wo: jax.Array,
    B_x: jax.Array,
    B_w1: jax.Array,
    B_b1: jax.Array,
    B_w2: jax.Array,
    B_b2: jax.Array,
    c: jax.Array,
    w_mod: jax.Array,
):
    del B_x
    nb, sq, d = A_x.shape
    _, nh, sk, dh = A_k_cache.shape
    f = B_w1.shape[1]
    win = min(4096, max(256, sk // 4))
    assert (nb, sq, dh, nh, win) == (4, 1, T, 32, RING * T) and d % T == 0
    dt = A_x.dtype
    ng = nh // 2
    hbm = pl.BlockSpec(memory_space=pltpu.HBM)
    dma = pltpu.SemaphoreType.DMA
    out = pl.pallas_call(
        functools.partial(_kernel, win=win),
        out_shape=jax.ShapeDtypeStruct((nb, d), dt),
        in_specs=[hbm] * 11,
        out_specs=pl.BlockSpec(memory_space=pltpu.VMEM),
        scratch_shapes=[
            pltpu.VMEM((nb, d), dt),
            pltpu.VMEM((nb, d), dt),
            pltpu.VMEM((f,), dt),
            pltpu.VMEM((d,), dt),
            pltpu.VMEM((RING, 2, 2, nb, T, dh), dt),
            pltpu.VMEM(A_wq.shape, dt),
            pltpu.VMEM(A_wo.shape, dt),
            pltpu.VMEM((f, d), dt),
            pltpu.VMEM((f, d), dt),
            pltpu.VMEM(w_mod.shape, dt),
            pltpu.VMEM((RING, 8, T), F32),
            pltpu.VMEM((8, d), F32),
            pltpu.VMEM((8, d), F32),
            pltpu.VMEM((8, 4 * d), F32),
            dma((RING,)), dma((ng,)), dma((ng,)), dma((7,)), dma((pl.cdiv(f, T),)),
        ],
        compiler_params=pltpu.CompilerParams(
            vmem_limit_bytes=64 * 2**20, disable_bounds_checks=True),
    )(A_x.reshape(nb, d), c, B_b1, B_b2, A_k_cache, A_v_cache, A_wq, A_wo, B_w1.T, B_w2, w_mod)
    return out.reshape(nb, sq, d)
```

```python
import functools

import jax
import jax.numpy as jnp
from jax import lax
import jax.experimental.pallas as pl
import jax.experimental.pallas.tpu as pltpu

F32 = jnp.float32
BF16 = jnp.bfloat16

T = 128
LOOK = 8
RING = 16
EPS = 1e-5
NOCOMP = 0
KVSHAPE = 1
NOSEMCHK = True
WQT = 3
WOT = 7
FCH = 32


def _nn(a, b):
    if NOCOMP:
        return jnp.zeros((a.shape[0], b.shape[1]), F32) + 1.0
    return lax.dot_general(a, b, (((1,), (0,)), ((), ())), preferred_element_type=F32)


def _nt(a, b):
    if NOCOMP:
        return jnp.zeros((a.shape[0], b.shape[0]), F32) + 1.0
    return lax.dot_general(a, b, (((1,), (1,)), ((), ())), preferred_element_type=F32)


def _layernorm(x):
    m = jnp.mean(x, axis=-1, keepdims=True)
    d = x - m
    v = jnp.mean(d * d, axis=-1, keepdims=True)
    return d * lax.rsqrt(v + EPS)


def _dup(x):
    return jnp.concatenate([x, x], axis=0)


def _kernel(x_hbm, c_hbm, b1_hbm, b2_hbm, k_hbm, v_hbm, wq_hbm, wo_hbm, w1t_hbm, w2_hbm, wm_hbm,
            out_ref,
            xb, cb, b1b, b2b, kv, wq, wo, w1t, w2, wm, s_ref, h_ref, y_ref, mod_ref,
            kv_sem, wq_sem, wo_sem, misc_sem, w2_sem, *, win):
    nb, nh, sk, dh = k_hbm.shape
    d = x_hbm.shape[1]
    f = w2_hbm.shape[0]
    ng = nh // 2
    nj = win // T
    row0 = sk - win
    nd = d // T
    scale = dh ** -0.5
    SM_X, SM_C, SM_B1, SM_B2, SM_MA, SM_MB, SM_W1 = range(7)
    mult = pl.multiple_of

    def kv_copy(which, g, j, t):
        src = (k_hbm, v_hbm)[which]
        if KVSHAPE == 0:
            hh, r = t // 4, (t % 4) * 32
            return pltpu.make_async_copy(
                src.at[:, 2 * g + hh, pl.ds(row0 + j * T + r, 32), :],
                kv.at[j, which, hh, :, pl.ds(r, 32), :], kv_sem.at[j])
        if KVSHAPE == 1:
            hh, r = t % 2, (t // 2) * 32
            return pltpu.make_async_copy(
                src.at[:, 2 * g + hh, pl.ds(row0 + j * T + r, 32), :],
                kv.at[j, which, hh, :, pl.ds(r, 32), :], kv_sem.at[j])
        b, r = t % 4, (t // 4) * 64
        return pltpu.make_async_copy(
            src.at[b, pl.ds(2 * g, 2), pl.ds(row0 + j * T + r, 64), :],
            kv.at[j, which, :, b, pl.ds(r, 64), :], kv_sem.at[j])

    def blk_copy(src, dst, sem, r, nr, c, nc):
        return pltpu.make_async_copy(src.at[pl.ds(r, nr), pl.ds(c, nc)],
                                     dst.at[pl.ds(r, nr), pl.ds(c, nc)], sem)

    def wq_copy(g, j):
        nr = 2 * d // nj
        return blk_copy(wq_hbm, wq, wq_sem.at[g % 2], mult((j // 2) * nr, 16), nr,
                        mult((2 * g + j % 2) * T, T), T)

    def wo_copy(g, j):
        return blk_copy(wo_hbm, wo, wo_sem.at[g % 4], mult((g * nj + j) * 16, 16), 16, 0, d)

    def wm_copy(cc, r, sem):
        return blk_copy(wm_hbm, wm, misc_sem.at[sem], mult(r * 16, 16), 16,
                        mult(cc * 2 * d, T), 2 * d)

    def wait_all(ref, sem):
        pltpu.make_async_copy(ref, ref, sem).wait()

    rows = lax.broadcasted_iota(jnp.int32, (8, T), 0)

    def step(j, carry, q, m, issue):
        mx, l, acc = carry
        if q is not None and m is not None:
            wait_all(kv.at[j], kv_sem.at[j])
        else:
            wait_all(kv.at[j, 0 if m is None else 1], kv_sem.at[j])
        if m is not None:
            p = jnp.exp(s_ref[j] - m)
            l = l + p
            p = p.astype(BF16)
        s = o = None
        for t in range(8):
            issue(t)
            if q is not None:
                r = _nt(q, kv[j, 0, t // 4, t % 4])
                s = r if s is None else jnp.where(rows == t, r, s)
            if m is not None:
                r = _nn(p, kv[j, 1, t // 4, t % 4])
                o = r if o is None else jnp.where(rows == t, r, o)
        if q is not None:
            s = s * scale
            s_ref[j] = s
            mx = jnp.maximum(mx, s)
        if m is not None:
            acc = acc + o
        return mx, l, acc

    def issue_first(j):
        def issue(t):
            kv_copy(0, 0, j, t).start(priority=int(t == 5))
            if t < 5:
                n = j * 5 + t
                wm_copy(1 + n % 2, n // 2, SM_MB).start(priority=1)
            elif t == 6:
                wq_copy(1, j).start(priority=1)
            elif t == 7:
                wo_copy(0, j).start(priority=1)
        return issue

    def issue_mid(g, j, last=False):
        def issue(t):
            kv_copy(0, g, j, t).start(priority=0)
            kv_copy(1, g - 1, j, t).start(priority=1)
            if t == WQT and not last:
                wq_copy(g + 1, j).start(priority=0)
            if t == WOT:
                wo_copy(g, j).start(priority=1)
        return issue

    def issue_last(j):
        def issue(t):
            kv_copy(1, ng - 1, j, (t % 2) * 4 + t // 2).start(priority=t % 2)
        return issue

    nfc = f // FCH
    fper = nfc // 3

    def issue_ffn(src, dst, sem_of, jj):
        def issue(t):
            for u in range(t * fper // 8, (t + 1) * fper // 8):
                n = jj * (fper // 2) + u // 2 + (u % 2) * (nfc // 2)
                blk_copy(src, dst, sem_of(jj), mult(n * FCH, FCH), FCH, 0, d).start(priority=u % 2)
        return issue

    def init():
        return (jnp.full((8, T), -jnp.inf, F32), jnp.zeros((8, T), F32), jnp.zeros((8, T), F32))

    def project_q(g):
        wq_g = wq.at[:, pl.ds(mult(2 * g * T, 2 * T), 2 * T)]
        wait_all(wq_g, wq_sem.at[g % 2])
        r = _nn(h_ref[...], wq_g[...])
        return jnp.where(rows < 4, r[:, :T], r[:, T:]).astype(BF16)

    def project_o(g, l, acc):
        wo_g = wo.at[pl.ds(mult(2 * g * T, 2 * T), 2 * T), :]
        wait_all(wo_g, wo_sem.at[g % 4])
        o = acc / jnp.sum(l, axis=-1, keepdims=True)
        o = jnp.concatenate([jnp.where(rows < 4, o, 0.0), jnp.where(rows < 4, 0.0, o)], axis=1)
        y_ref[...] += _nn(o.astype(BF16), wo_g[...])

    def rowmax(mx):
        return jnp.max(mx, axis=-1, keepdims=True)

    nra = d // 16

    def mod_a_start(n, _):
        wm_copy(0, n, SM_MA).start(priority=0)
        wm_copy(0, n + nra // 2, SM_MA).start(priority=1)
        return _

    mod_a_start(0, 0)
    small = [pltpu.make_async_copy(s, t, misc_sem.at[i]) for s, t, i in
             ((x_hbm, xb, SM_X), (c_hbm, cb, SM_C), (b1_hbm, b1b, SM_B1), (b2_hbm, b2b, SM_B2))]
    for cp in small:
        cp.start()
    lax.fori_loop(1, nra // 2, mod_a_start, 0)

    def first_wq(j, _):
        wq_copy(0, j).start(priority=0)
        wq_copy(0, j + nj // 2).start(priority=1)
        return _

    lax.fori_loop(0, nj // 2, first_wq, 0)

    def first_issue(j, _):
        for t in range(8):
            issue_first(j)(t)
        return _

    lax.fori_loop(0, LOOK, first_issue, 0)

    for cp in small:
        cp.wait()
    wait_all(wm.at[:, pl.ds(0, 2 * d)], misc_sem.at[SM_MA])
    x = _dup(xb[...].astype(F32))
    cf = _dup(cb[...].astype(F32))
    sc = (cf * jax.nn.sigmoid(cf)).astype(BF16)
    mod_a = _nn(sc, wm[:, 0:2 * d])
    h_ref[...] = (_layernorm(x) * (1.0 + mod_a[:, d:]) + mod_a[:, :d]).astype(BF16)
    y_ref[...] = jnp.zeros_like(y_ref)

    q = project_q(0)
    carry = lax.fori_loop(
        0, nj - LOOK, lambda j, cr: step(j, cr, q, None, issue_first(j + LOOK)), init())
    carry = lax.fori_loop(
        nj - LOOK, nj, lambda j, cr: step(j, cr, q, None, issue_mid(1, j + LOOK - nj)), carry)

    wait_all(wm.at[:, pl.ds(2 * d, 4 * d)], misc_sem.at[SM_MB])
    mod_ref[...] = _nn(sc, wm[:, 2 * d:])

    def phase(g, carry, last_next=False):
        mx, l, acc = carry
        q = project_q(g)
        if isinstance(g, int):
            project_o(g - 2, l, acc)
        else:
            pl.when(g >= 2)(lambda: project_o(g - 2, l, acc))
        m = rowmax(mx)
        last = isinstance(g, int) and g == ng - 1
        carry = lax.fori_loop(
            0, nj - LOOK, lambda j, cr: step(j, cr, q, m, issue_mid(g, j + LOOK, last)), init())
        nxt = issue_last if last else functools.partial(issue_mid, g + 1, last=last_next)
        return lax.fori_loop(
            nj - LOOK, nj, lambda j, cr: step(j, cr, q, m, nxt(j + LOOK - nj)), carry)

    carry = lax.fori_loop(1, ng - 2, phase, carry)
    carry = phase(ng - 2, carry, last_next=True)
    mx, l, acc = phase(ng - 1, carry)

    project_o(ng - 2, l, acc)
    m = rowmax(mx)
    j0 = nj - LOOK
    carry = lax.fori_loop(
        0, j0, lambda j, cr: step(j, cr, None, m, issue_last(j + LOOK)), init())
    carry = lax.fori_loop(
        j0, j0 + 3, lambda j, cr: step(
            j, cr, None, m, issue_ffn(w1t_hbm, w1t, lambda _: misc_sem.at[SM_W1], j - j0)), carry)
    carry = lax.fori_loop(
        j0 + 3, j0 + 6, lambda j, cr: step(
            j, cr, None, m, issue_ffn(w2_hbm, w2, lambda jj: w2_sem.at[jj], j - j0 - 3)), carry)
    mx, l, acc = lax.fori_loop(
        j0 + 6, nj, lambda j, cr: step(j, cr, None, m, lambda t: None), carry)
    project_o(ng - 1, l, acc)

    y = y_ref[...]
    y = y + pltpu.roll(y, 4, 0)
    ga, sb, cbm, gb = (mod_ref[:, i * d:(i + 1) * d] for i in range(4))
    x1 = x + ga * y
    h2 = (_layernorm(x1) * (1.0 + cbm) + sb).astype(BF16)
    wait_all(w1t, misc_sem.at[SM_W1])
    nr = f // 6
    z = jnp.broadcast_to(b2b[...].astype(F32).reshape(1, d), (8, d))
    b1 = b1b[...].astype(F32).reshape(1, f)
    a = []
    for i in range(6):
        u = _nt(h2, w1t[i * nr:(i + 1) * nr, :]) + b1[:, i * nr:(i + 1) * nr]
        a.append(jax.nn.gelu(u, approximate=True).astype(BF16))
    for jj in range(3):
        wait_all(w2.at[pl.ds(0, 2 * nr), :], w2_sem.at[jj])
        for i in (jj, jj + 3):
            z = z + _nn(a[i], w2[i * nr:(i + 1) * nr, :])
    out_ref[...] = (x1 + gb * z)[0:4].astype(out_ref.dtype)


@jax.jit
def pallas_adaLN_cond__sliding_block_cached__dense_activation_gelu__decode_kernel(
    A_x: jax.Array,
    A_k_cache: jax.Array,
    A_v_cache: jax.Array,
    A_wq: jax.Array,
    A_wo: jax.Array,
    B_x: jax.Array,
    B_w1: jax.Array,
    B_b1: jax.Array,
    B_w2: jax.Array,
    B_b2: jax.Array,
    c: jax.Array,
    w_mod: jax.Array,
):
    del B_x
    nb, sq, d = A_x.shape
    _, nh, sk, dh = A_k_cache.shape
    f = B_w1.shape[1]
    win = min(4096, max(256, sk // 4))
    assert (nb, sq, dh, nh, win) == (4, 1, T, 32, RING * T) and d % T == 0
    dt = A_x.dtype
    hbm = pl.BlockSpec(memory_space=pltpu.HBM)
    dma = pltpu.SemaphoreType.DMA
    out = pl.pallas_call(
        functools.partial(_kernel, win=win),
        out_shape=jax.ShapeDtypeStruct((nb, d), dt),
        in_specs=[hbm] * 11,
        out_specs=pl.BlockSpec(memory_space=pltpu.VMEM),
        scratch_shapes=[
            pltpu.VMEM((nb, d), dt),
            pltpu.VMEM((nb, d), dt),
            pltpu.VMEM((f,), dt),
            pltpu.VMEM((d,), dt),
            pltpu.VMEM((RING, 2, 2, nb, T, dh), dt),
            pltpu.VMEM(A_wq.shape, dt),
            pltpu.VMEM(A_wo.shape, dt),
            pltpu.VMEM((f, d), dt),
            pltpu.VMEM((f, d), dt),
            pltpu.VMEM(w_mod.shape, dt),
            pltpu.VMEM((RING, 8, T), F32),
            pltpu.VMEM((8, d), dt),
            pltpu.VMEM((8, d), F32),
            pltpu.VMEM((8, 4 * d), F32),
            dma((RING,)), dma((2,)), dma((4,)), dma((7,)), dma((3,)),
        ],
        compiler_params=pltpu.CompilerParams(
            vmem_limit_bytes=64 * 2**20, disable_bounds_checks=True,
            disable_semaphore_checks=NOSEMCHK),
    )(A_x.reshape(nb, d), c, B_b1, B_b2, A_k_cache, A_v_cache, A_wq, A_wo, B_w1.T, B_w2, w_mod)
    return out.reshape(nb, sq, d)
```

```python
import functools

import jax
import jax.numpy as jnp
from jax import lax
import jax.experimental.pallas as pl
import jax.experimental.pallas.tpu as pltpu

F32 = jnp.float32
BF16 = jnp.bfloat16

T = 128
NJ = 16
LOOK = 8
EPS = 1e-5
W2_CUTS = (3, 5)


def _nn(a, b):
    return lax.dot_general(a, b, (((1,), (0,)), ((), ())), preferred_element_type=F32)


def _nt(a, b):
    return lax.dot_general(a, b, (((1,), (1,)), ((), ())), preferred_element_type=F32)


def _layernorm(x):
    m = jnp.mean(x, axis=-1, keepdims=True)
    d = x - m
    v = jnp.mean(d * d, axis=-1, keepdims=True)
    return d * lax.rsqrt(v + EPS)


def _dup(x):
    return jnp.concatenate([x, x], axis=0)


def _kernel(x_hbm, c_hbm, b1_hbm, b2_hbm, k_hbm, v_hbm, wq_hbm, wo_hbm, w1t_hbm, w2_hbm, wm_hbm,
            out_ref,
            xb, cb, b1b, b2b, kv, wq, wo, w1t, w2, wm, s_ref, h_ref, y_ref, mod_ref,
            kv_sem, wq_sem, wo_sem, w2_sem):
    _, nh, sk, dh = k_hbm.shape
    d = x_hbm.shape[1]
    f = w2_hbm.shape[0]
    ng = nh // 2
    row0 = sk - NJ * T
    scale = dh ** -0.5
    mult = pl.multiple_of
    small_sem, ma_sem, mb_sem, w1_sem = w2_sem.at[0], w2_sem.at[1], w2_sem.at[2], wq_sem.at[0]

    def kv_copy(which, g, j, t, by_batch=False):
        src = (k_hbm, v_hbm)[which]
        sem = kv_sem.at[j % LOOK]
        if not by_batch:
            hh, r = t % 2, (t // 2) * 32
            return pltpu.make_async_copy(
                src.at[:, 2 * g + hh, pl.ds(row0 + j * T + r, 32), :],
                kv.at[j, which, hh, :, pl.ds(r, 32), :], sem)
        b, r = t % 4, (t // 4) * 64
        return pltpu.make_async_copy(
            src.at[b, pl.ds(2 * g, 2), pl.ds(row0 + j * T + r, 64), :],
            kv.at[j, which, :, b, pl.ds(r, 64), :], sem)

    def blk_copy(src, dst, sem, i, nr, c, nc):
        r = mult(i * nr, nr)
        return pltpu.make_async_copy(src.at[pl.ds(r, nr), pl.ds(c, nc)],
                                     dst.at[pl.ds(r, nr), pl.ds(c, nc)], sem)

    nq = d // 64
    no = 2 * dh // 32

    def wq_copy(g, i):
        return blk_copy(wq_hbm, wq, wq_sem.at[g % 2], i, 64, mult(g * 2 * dh, 2 * dh), 2 * dh)

    def wo_copy(g, i):
        return blk_copy(wo_hbm, wo, wo_sem.at[g % 2], g * no + i, 32, 0, d)

    def wm_copy(cc, i, sem):
        return blk_copy(wm_hbm, wm, sem, i, 16, mult(cc * 2 * d, T), 2 * d)

    def wait_all(ref, sem):
        pltpu.make_async_copy(ref, ref, sem).wait()

    def start_proj(g, j):
        if not (isinstance(g, int) and g == ng - 1):
            pl.when(j < nq)(lambda: wq_copy(g + 1, j).start(priority=0))
        pl.when(j >= NJ - no)(lambda: wo_copy(g, j - (NJ - no)).start(priority=1))

    nmb = 2 * (d // 16) // NJ

    def issue_first(j):
        def issue(t):
            kv_copy(0, 0, j, t).start(priority=int(t > nmb))
            if t < nmb:
                n = j * nmb + t
                wm_copy(1 + n % 2, n // 2, mb_sem).start(priority=1)
            if t == nmb:
                start_proj(0, j)
        return issue

    def issue_mid(g, j):
        def issue(t):
            kv_copy(0, g, j, t).start(priority=0)
            kv_copy(1, g - 1, j, t).start(priority=1)
            if t == 3:
                start_proj(g, j)
        return issue

    def issue_last(j):
        def issue(t):
            kv_copy(1, ng - 1, j, (0, 6, 1, 7, 4, 2, 5, 3)[t], True).start(priority=t % 2)
        return issue

    nfp = f // 32
    nfs = 3
    nfc = pl.cdiv(f, T)
    half = pl.cdiv(nfc, 2)

    def w2_span(chunk):
        side = (chunk >= half).astype(jnp.int32)
        i = chunk - side * half
        return side + 2 * sum((i >= cut).astype(jnp.int32) for cut in W2_CUTS)

    def issue_mlp(src, dst, sem_of, jj):
        per = nfp // nfs

        def issue(t):
            for u in range(t * per // 8, (t + 1) * per // 8):
                n = jj * (per // 2) + u // 2 + (u % 2) * (nfp // 2)
                blk_copy(src, dst, sem_of(n), n, 32, 0, d).start(priority=u % 2)
        return issue

    rows = lax.broadcasted_iota(jnp.int32, (8, T), 0)

    def step(j, carry, q, m, issue):
        mx, l, acc = carry
        both = q is not None and m is not None
        wait_all(kv.at[j] if both else kv.at[j, 0 if m is None else 1], kv_sem.at[j % LOOK])
        if m is not None:
            p = jnp.exp(s_ref[j] - m)
            l = l + p
            p = p.astype(BF16)
        s = o = None
        for t in range(8):
            issue(t)
            if q is not None:
                r = _nt(q, kv[j, 0, t // 4, t % 4])
                s = r if s is None else jnp.where(rows == t, r, s)
            if m is not None:
                r = _nn(p, kv[j, 1, t // 4, t % 4])
                o = r if o is None else jnp.where(rows == t, r, o)
        if q is not None:
            s = s * scale
            s_ref[j] = s
            mx = jnp.maximum(mx, s)
        if m is not None:
            acc = acc + o
        return mx, l, acc

    def steps(lo, hi, carry, q, m, issue_of):
        return lax.fori_loop(lo, hi, lambda j, cr: step(j, cr, q, m, issue_of(j)), carry)

    def init():
        return (jnp.full((8, T), -jnp.inf, F32), jnp.zeros((8, T), F32), jnp.zeros((8, T), F32))

    def project_q(g):
        wq_g = wq.at[:, pl.ds(mult(g * 2 * dh, 2 * dh), 2 * dh)]
        wait_all(wq_g, wq_sem.at[g % 2])
        r = _nn(h_ref[...], wq_g[...])
        return jnp.where(rows < 4, r[:, :dh], r[:, dh:]).astype(BF16)

    def project_o(g, l, acc):
        wo_g = wo.at[pl.ds(mult(g * 2 * dh, 2 * dh), 2 * dh), :]
        wait_all(wo_g, wo_sem.at[g % 2])
        o = acc / jnp.sum(l, axis=-1, keepdims=True)
        o = jnp.concatenate([jnp.where(rows < 4, o, 0.0), jnp.where(rows < 4, 0.0, o)], axis=1)
        y_ref[...] += _nn(o.astype(BF16), wo_g[...])

    def rowmax(mx):
        return jnp.max(mx, axis=-1, keepdims=True)

    nma = d // 16

    def start_mod_a(i, carry):
        wm_copy(0, i, ma_sem).start(priority=0)
        wm_copy(0, i + nma // 2, ma_sem).start(priority=1)
        return carry

    start_mod_a(0, 0)
    small = [pltpu.make_async_copy(s, t, small_sem)
             for s, t in ((x_hbm, xb), (c_hbm, cb), (b1_hbm, b1b), (b2_hbm, b2b))]
    for cp in small:
        cp.start()
    lax.fori_loop(1, nma // 2, start_mod_a, 0)
    for i in range(nq // 2):
        wq_copy(0, i).start(priority=0)
        wq_copy(0, i + nq // 2).start(priority=1)

    def start_first(j, carry):
        for t in range(8):
            issue_first(j)(t)
        return carry

    lax.fori_loop(0, LOOK, start_first, 0)

    for cp in small:
        cp.wait()
    wait_all(wm.at[:, pl.ds(0, 2 * d)], ma_sem)
    x = _dup(xb[...].astype(F32))
    cf = _dup(cb[...].astype(F32))
    sc = (cf * jax.nn.sigmoid(cf)).astype(BF16)
    mod_a = _nn(sc, wm[:, 0:2 * d])
    h_ref[...] = (_layernorm(x) * (1.0 + mod_a[:, d:]) + mod_a[:, :d]).astype(BF16)
    y_ref[...] = jnp.zeros_like(y_ref)

    j0 = NJ - LOOK
    q = project_q(0)
    carry = steps(0, j0, init(), q, None, lambda j: issue_first(j + LOOK))
    carry = steps(j0, NJ, carry, q, None, lambda j: issue_mid(1, j - j0))
    wait_all(wm.at[:, pl.ds(2 * d, 4 * d)], mb_sem)
    mod_ref[...] = _nn(sc, wm[:, 2 * d:])

    def phase(g, carry):
        mx, l, acc = carry
        static = isinstance(g, int)
        q = project_q(g)
        if static:
            project_o(g - 2, l, acc)
        else:
            pl.when(g >= 2)(lambda: project_o(g - 2, l, acc))
        m = rowmax(mx)
        carry = steps(0, j0, init(), q, m, lambda j: issue_mid(g, j + LOOK))
        nxt = issue_last if static and g == ng - 1 else functools.partial(issue_mid, g + 1)
        return steps(j0, NJ, carry, q, m, lambda j: nxt(j - j0))

    carry = lax.fori_loop(1, ng - 2, phase, carry)
    carry = phase(ng - 2, carry)
    mx, l, acc = phase(ng - 1, carry)

    project_o(ng - 2, l, acc)
    m = rowmax(mx)
    carry = steps(0, j0, init(), None, m, lambda j: issue_last(j + LOOK))
    carry = steps(j0, j0 + nfs, carry, None, m,
                  lambda j: issue_mlp(w1t_hbm, w1t, lambda n: w1_sem, j - j0))
    carry = steps(j0 + nfs, j0 + 2 * nfs, carry, None, m,
                  lambda j: issue_mlp(w2_hbm, w2, lambda n: w2_sem.at[w2_span(n >> 2)],
                                      j - j0 - nfs))
    mx, l, acc = steps(j0 + 2 * nfs, NJ, carry, None, m, lambda j: lambda t: None)
    project_o(ng - 1, l, acc)

    y = y_ref[...]
    y = y + pltpu.roll(y, 4, 0)
    ga, sb, cbm, gb = (mod_ref[:, i * d:(i + 1) * d] for i in range(4))
    x1 = x + ga * y
    h2 = (_layernorm(x1) * (1.0 + cbm) + sb).astype(BF16)
    wait_all(w1t, w1_sem)
    a = _nt(h2, w1t[...]) + b1b[...].astype(F32).reshape(1, f)
    a = jax.nn.gelu(a, approximate=True).astype(BF16)
    z = jnp.broadcast_to(b2b[...].astype(F32).reshape(1, d), (8, d))
    for stage, (lo, hi) in enumerate(zip((0,) + W2_CUTS, W2_CUTS + (half,))):
        spans = [((side * half + lo) * T, min((side * half + hi) * T, f)) for side in range(2)]
        for side, (r0, r1) in enumerate(spans):
            wait_all(w2.at[pl.ds(r0, r1 - r0), :], w2_sem.at[2 * stage + side])
        for r0, r1 in spans:
            z = z + _nn(a[:, r0:r1], w2[r0:r1, :])
    out_ref[...] = (x1 + gb * z)[0:4].astype(out_ref.dtype)


@jax.jit
def pallas_adaLN_cond__sliding_block_cached__dense_activation_gelu__decode_kernel(
    A_x: jax.Array,
    A_k_cache: jax.Array,
    A_v_cache: jax.Array,
    A_wq: jax.Array,
    A_wo: jax.Array,
    B_x: jax.Array,
    B_w1: jax.Array,
    B_b1: jax.Array,
    B_w2: jax.Array,
    B_b2: jax.Array,
    c: jax.Array,
    w_mod: jax.Array,
):
    del B_x
    nb, sq, d = A_x.shape
    _, nh, sk, dh = A_k_cache.shape
    f = B_w1.shape[1]
    win = min(4096, max(256, sk // 4))
    assert (nb, sq, d, f, nh, dh, win) == (4, 1, 640, 1728, 32, T, NJ * T)
    dt = A_x.dtype
    hbm = pl.BlockSpec(memory_space=pltpu.HBM)
    dma = pltpu.SemaphoreType.DMA
    out = pl.pallas_call(
        _kernel,
        out_shape=jax.ShapeDtypeStruct((nb, d), dt),
        in_specs=[hbm] * 11,
        out_specs=pl.BlockSpec(memory_space=pltpu.VMEM),
        scratch_shapes=[
            pltpu.VMEM((nb, d), dt),
            pltpu.VMEM((nb, d), dt),
            pltpu.VMEM((f,), dt),
            pltpu.VMEM((d,), dt),
            pltpu.VMEM((NJ, 2, 2, nb, T, dh), dt),
            pltpu.VMEM(A_wq.shape, dt),
            pltpu.VMEM(A_wo.shape, dt),
            pltpu.VMEM((f, d), dt),
            pltpu.VMEM((f, d), dt),
            pltpu.VMEM(w_mod.shape, dt),
            pltpu.VMEM((NJ, 8, T), F32),
            pltpu.VMEM((8, d), dt),
            pltpu.VMEM((8, d), F32),
            pltpu.VMEM((8, 4 * d), F32),
            dma((LOOK,)), dma((2,)), dma((2,)), dma((6,)),
        ],
        compiler_params=pltpu.CompilerParams(vmem_limit_bytes=64 * 2**20),
    )(A_x.reshape(nb, d), c, B_b1, B_b2, A_k_cache, A_v_cache, A_wq, A_wo, B_w1.T, B_w2, w_mod)
    return out.reshape(nb, sq, d)
```
